```python
import os as _os
_os.environ.setdefault("JAX_PLATFORMS", "cpu")
import jax
import jax.numpy as jnp

def _softmax(x, axis=-1):
    return jax.nn.softmax(x, axis=axis)
def _gelu(x):
    return jax.nn.gelu(x, approximate=True)
def _silu(x):
    return jax.nn.silu(x)
def _sigmoid(x):
    return jax.nn.sigmoid(x)
def _layernorm(x, axis=-1, eps=1e-5):
    m = jnp.mean(x, axis=axis, keepdims=True)
    v = jnp.var(x, axis=axis, keepdims=True)
    return (x - m) / jnp.sqrt(v + eps)
def _scatter_add(tgt, idx, src, axis=0):
    return tgt.at[idx].add(src)
def _segment_sum(src, seg, n):
    return jax.ops.segment_sum(src, seg, n)
class _Rng:
    def __init__(self, key):
        self._k = key
    def _next(self):
        self._k, sub = jax.random.split(self._k)
        return sub
    def normal(self, shape):
        return jax.random.normal(self._next(), shape, dtype=jnp.bfloat16)
    def randint(self, lo, hi, shape):
        return jax.random.randint(self._next(), shape, lo, hi, dtype=jnp.int32)
    def uniform(self, shape, lo=0.0, hi=1.0):
        return jax.random.uniform(self._next(), shape, jnp.bfloat16, lo, hi)
    def permutation(self, n):
        return jax.random.permutation(self._next(), n)


kernel_name = 'sequential_preLN__linear_kernel_hedgehog__geglu_ffn__prompt'

def setup_inputs():
    _rng = _Rng(jax.random.key(int.from_bytes(__import__("os").urandom(4), "little")))
    _w = (lambda a: (lambda t: t.astype(jnp.bfloat16) if jnp.issubdtype(t.dtype, jnp.floating) else t)(jnp.asarray(a)))
    def _A_setup():
        B, S, D, H = 1, 2048, 640, 32
        Dh = D // H
        return {
            "x": _w((lambda *s: _rng.normal(s) * 0.05)(B, S, D)),
            "wqkv": _w((lambda *s: _rng.normal(s) * 0.2)(D, 3 * D)),
            "w_phi": _w((lambda *s: _rng.normal(s) * 0.2)(H, Dh, Dh) * (Dh ** -0.5)),
            "wo": _w((lambda *s: _rng.normal(s) * 0.05)(D, D)),
        }
    _A_in = _A_setup()

    def _B_setup():
        B, S, D, F = 1, 2048, 640, 1536
        return {
            "x": _w((lambda *s: _rng.normal(s) * 0.05)(B, S, D)),
            "w_gate": _w((lambda *s: _rng.normal(s) * 0.05)(D, F)),
            "w_up": _w((lambda *s: _rng.normal(s) * 0.05)(D, F)),
            "w_down": _w((lambda *s: _rng.normal(s) * 0.05)(F, D)),
        }
    _B_in = _B_setup()

    return {
        "A_x": _A_in["x"],
        "A_wqkv": _A_in["wqkv"],
        "A_w_phi": _A_in["w_phi"],
        "A_wo": _A_in["wo"],
        "B_x": _B_in["x"],
        "B_w_gate": _B_in["w_gate"],
        "B_w_up": _B_in["w_up"],
        "B_w_down": _B_in["w_down"],
    }

def reference(A_x, A_wqkv, A_w_phi, A_wo, B_x, B_w_gate, B_w_up, B_w_down):
    def _A_ref(x, wqkv, w_phi, wo):
        B, S, D = x.shape
        H = 32; Dh = D // H
        qkv = (lambda x, *d: x.transpose(*d))((x @ wqkv).reshape(B, S, 3, H, Dh), 2, 0, 3, 1, 4)
        q, k, v = qkv[0], qkv[1], qkv[2]
        pq = jnp.einsum("bhsd,hdf->bhsf", q, w_phi)
        pk = jnp.einsum("bhsd,hdf->bhsf", k, w_phi)
        phi_q = jnp.concatenate([_softmax(pq, axis=-1), _softmax(-pq, axis=-1)], axis=-1)
        phi_k = jnp.concatenate([_softmax(pk, axis=-1), _softmax(-pk, axis=-1)], axis=-1)
        kv = jnp.einsum("bhsf,bhsd->bhfd", phi_k, v)
        z  = jnp.einsum("bhsf->bhf", phi_k)
        num = jnp.einsum("bhqf,bhfd->bhqd", phi_q, kv)
        den = jnp.einsum("bhqf,bhf->bhq", phi_q, z)[..., None] + 1e-6
        o = num / den
        return (lambda x, *d: x.transpose(*d))(o, 0, 2, 1, 3).reshape(B, S, D) @ wo

    def _B_ref(x, w_gate, w_up, w_down):
        return (_gelu(x @ w_gate) * (x @ w_up)) @ w_down

    x = A_x
    h = x + _A_ref(_layernorm(x, axis=-1), A_wqkv, A_w_phi, A_wo)
    h2 = h + _B_ref(_layernorm(h, axis=-1), B_w_gate, B_w_up, B_w_down)
    return h2
```

```python
import functools
import math

import jax
import jax.numpy as jnp
from jax import lax
import jax.experimental.pallas as pl
import jax.experimental.pallas.tpu as pltpu

F32 = jnp.float32
BF16 = jnp.bfloat16

NUM_HEADS = 32
HPG = 4
LN_EPS = 1e-5
DEN_EPS = 1e-6
LOG2E = math.log2(math.e)

T1 = 256
T2 = 256
FC = 512

_NN = (((1,), (0,)), ((), ()))
_NT = (((1,), (1,)), ((), ()))


def _dot(a, b, dims=_NN):
    return lax.dot_general(a, b, dims, preferred_element_type=F32)


def _iota(shape, dim):
    return lax.broadcasted_iota(jnp.int32, shape, dim)


def _idiv(v, n):
    return ((v.astype(F32) + 0.5) * (1.0 / n)).astype(jnp.int32)


def _layernorm(x):
    m = jnp.mean(x, axis=-1, keepdims=True)
    d = x - m
    var = jnp.mean(d * d, axis=-1, keepdims=True)
    return d * lax.rsqrt(var + LN_EPS)


def _gelu(x):
    c = math.sqrt(2.0 / math.pi)
    inner = x * (c + (c * 0.044715) * (x * x))
    return (0.5 * x) * (1.0 + jnp.tanh(inner))


def _all_reduce(v, op):
    return op(v, pltpu.roll(v, HPG, 0))


def _dual_exp(p):
    rows, t = p.shape
    p3 = p.reshape(rows // 8, 8, t)
    mx = _all_reduce(jnp.max(p3, axis=0), jnp.maximum)
    mn = _all_reduce(jnp.min(p3, axis=0), jnp.minimum)
    e_pos = jnp.exp2(p3 - mx[None])
    e_neg = jnp.exp2(mn[None] - p3)
    s_pos = _all_reduce(jnp.sum(e_pos, axis=0), jnp.add)
    s_neg = _all_reduce(jnp.sum(e_neg, axis=0), jnp.add)
    return e_pos, e_neg, s_pos, s_neg


def _pack(e_pos, e_neg, r_pos, r_neg):
    n, _, t = e_pos.shape
    a = (e_pos * r_pos[None]).reshape(n * 8, t)
    b = (e_neg * r_neg[None]).reshape(n * 8, t)
    return jnp.concatenate([a, b], axis=0).astype(BF16)


def _kernel(x_hbm, wqkv_hbm, wphi_ref, wo_hbm, wg_hbm, wu_hbm, wd_hbm, out_hbm,
            x_v, xn_v, wqkv_v, wt_v, wo_v, wg_v, wu_v, wd_v, out_v,
            phi_v, kv_acc, kvt_v, z_v, x_sem, w_sem, o_sem):
    S, D = x_v.shape
    F = wg_v.shape[1]
    Dh = D // NUM_HEADS
    G = NUM_HEADS // HPG
    GR = HPG * Dh
    n1, n2 = S // T1, S // T2

    def x_copy(t):
        rows = pl.ds(t * T1, T1)
        return pltpu.make_async_copy(x_hbm.at[rows], x_v.at[rows], x_sem.at[t])

    def wqkv_copy(j):
        cols = pl.ds(j * D, D)
        return pltpu.make_async_copy(wqkv_hbm.at[:, cols], wqkv_v.at[j], w_sem.at[j])

    wo_copy = pltpu.make_async_copy(wo_hbm, wo_v, w_sem.at[3])
    wg_copy = pltpu.make_async_copy(wg_hbm, wg_v, w_sem.at[4])
    wu_copy = pltpu.make_async_copy(wu_hbm, wu_v, w_sem.at[5])
    wd_copy = pltpu.make_async_copy(wd_hbm, wd_v, w_sem.at[6])

    wqkv_copy(1).start()
    wqkv_copy(2).start()
    x_copy(0).start()

    phi_v[...] = jnp.zeros(phi_v.shape, F32)
    for h in range(NUM_HEADS):
        phi_v[h * Dh:(h + 1) * Dh, 0:Dh] = wphi_ref[h].astype(F32)
    SR = 2 * GR
    r = _iota((SR, 128), 0)
    r_grp = _idiv(r, GR)
    r_f = (r - r_grp * GR) >> 2
    sel = (r_f == _iota((SR, 128), 1)).astype(BF16)
    r2 = _iota((SR, 256), 0)
    r_head = _idiv(r2, GR) * HPG + (r2 & (HPG - 1))
    c2 = _iota((SR, 256), 1)
    pts = []
    for b in range(G // 2):
        blk = phi_v[b * 128:b * 128 + 256, :].astype(BF16)
        full = _dot(sel, blk, _NT)
        keep = (r_head + b * 2 * HPG) == _idiv(c2 + b * 128, Dh)
        pts.append(jnp.where(keep, full, 0.0).astype(BF16))

    def fold(j):
        for b in range(G // 2):
            w = wqkv_v[j, :, b * 128:b * 128 + 256]
            wt_v[j, b * SR:(b + 1) * SR, :] = (_dot(pts[b], w, _NT) * LOG2E).astype(BF16)

    wqkv_copy(1).wait()
    for t in range(1, n1):
        x_copy(t).start()
    wqkv_copy(0).start()
    fold(1)
    wqkv_copy(2).wait()
    wo_copy.start()
    wg_copy.start()
    wu_copy.start()
    wd_copy.start()
    wt_v[2] = wqkv_v[2].T
    wqkv_copy(0).wait()
    fold(0)

    kv_acc[...] = jnp.zeros(kv_acc.shape, F32)

    def kv_step(t, carry):
        x_copy(t).wait()
        rows = pl.ds(pl.multiple_of(t * T1, T1), T1)
        xn = _layernorm(x_v[rows, :].astype(F32)).astype(BF16)
        xn_v[rows, :] = xn
        pk = _dot(wt_v[1], xn, _NT)
        vt = _dot(wt_v[2], xn, _NT).astype(BF16)
        ones = jnp.ones((16, T1), BF16)
        for g in range(G):
            e_pos, e_neg, s_pos, s_neg = _dual_exp(pk[g * GR:(g + 1) * GR])
            phi = _pack(e_pos, e_neg, 1.0 / s_pos, 1.0 / s_neg)
            v1 = jnp.concatenate([vt[g * GR:(g + 1) * GR], ones], axis=0)
            kv_acc[g] += _dot(phi, v1, _NT)
        return carry

    lax.fori_loop(0, n1, kv_step, 0)

    keep = (_iota((SR, GR), 0) & (HPG - 1)) == _idiv(_iota((SR, GR), 1), Dh)
    for g in range(G):
        acc = kv_acc[g]
        kvt_v[g] = jnp.where(keep, acc[:, 0:GR], 0.0).T.astype(BF16)
        z_v[g] = jnp.broadcast_to(acc[:, GR:GR + 1], (SR, 128))

    wo_copy.wait()
    wg_copy.wait()
    wu_copy.wait()
    wd_copy.wait()

    def out_copy(t):
        rows = pl.ds(pl.multiple_of(t * T2, T2), T2)
        return pltpu.make_async_copy(out_v.at[rows], out_hbm.at[rows], o_sem.at[t])

    def q_step(t, carry):
        rows = pl.ds(pl.multiple_of(t * T2, T2), T2)
        pq = _dot(wt_v[0], xn_v[rows, :], _NT)
        ots = []
        for g in range(G):
            e_pos, e_neg, s_pos, s_neg = _dual_exp(pq[g * GR:(g + 1) * GR])
            z = jnp.concatenate([z_v[g]] * (T2 // 128), axis=1).reshape(SR // 8, 8, T2)
            d_pos = _all_reduce(jnp.sum(e_pos * z[:GR // 8], axis=0), jnp.add)
            d_neg = _all_reduce(jnp.sum(e_neg * z[GR // 8:], axis=0), jnp.add)
            r_pos, r_neg = 1.0 / s_pos, 1.0 / s_neg
            r_den = 1.0 / (d_pos * r_pos + d_neg * r_neg + DEN_EPS)
            phi = _pack(e_pos, e_neg, r_pos * r_den, r_neg * r_den)
            ots.append(_dot(kvt_v[g], phi).astype(BF16))
        o = jnp.concatenate(ots, axis=0).T
        h = x_v[rows, :].astype(F32) + _dot(o, wo_v[...])
        hn = _layernorm(h).astype(BF16)
        acc = h
        for c in range(F // FC):
            cols = slice(c * FC, (c + 1) * FC)
            act = _gelu(_dot(hn, wg_v[:, cols])) * _dot(hn, wu_v[:, cols])
            acc = acc + _dot(act.astype(BF16), wd_v[cols, :])
        out_v[rows, :] = acc.astype(out_v.dtype)
        out_copy(t).start()
        return carry

    lax.fori_loop(0, n2, q_step, 0)
    for t in range(n2):
        out_copy(t).wait()


@jax.jit
def pallas_sequential_preLN__linear_kernel_hedgehog__geglu_ffn__prompt_kernel(
    A_x: jax.Array,
    A_wqkv: jax.Array,
    A_w_phi: jax.Array,
    A_wo: jax.Array,
    B_x: jax.Array,
    B_w_gate: jax.Array,
    B_w_up: jax.Array,
    B_w_down: jax.Array,
):
    del B_x
    B, S, D = A_x.shape
    assert B == 1
    F = B_w_gate.shape[1]
    G = NUM_HEADS // HPG
    GR = D // G
    any_spec = pl.BlockSpec(memory_space=pl.ANY)
    out = pl.pallas_call(
        _kernel,
        out_shape=jax.ShapeDtypeStruct((S, D), A_x.dtype),
        in_specs=[any_spec, any_spec, pl.BlockSpec(memory_space=pltpu.VMEM),
                  any_spec, any_spec, any_spec, any_spec],
        out_specs=any_spec,
        scratch_shapes=[
            pltpu.VMEM((S, D), A_x.dtype),
            pltpu.VMEM((S, D), BF16),
            pltpu.VMEM((3, D, D), BF16),
            pltpu.VMEM((3, D, D), BF16),
            pltpu.VMEM((D, D), BF16),
            pltpu.VMEM((D, F), BF16),
            pltpu.VMEM((D, F), BF16),
            pltpu.VMEM((F, D), BF16),
            pltpu.VMEM((S, D), A_x.dtype),
            pltpu.VMEM((D, 128), F32),
            pltpu.VMEM((G, 2 * GR, GR + 16), F32),
            pltpu.VMEM((G, GR, 2 * GR), BF16),
            pltpu.VMEM((G, 2 * GR, 128), F32),
            pltpu.SemaphoreType.DMA((S // T1,)),
            pltpu.SemaphoreType.DMA((7,)),
            pltpu.SemaphoreType.DMA((S // T2,)),
        ],
        compiler_params=pltpu.CompilerParams(vmem_limit_bytes=100 * 1024 * 1024),
    )(A_x.reshape(S, D), A_wqkv, A_w_phi, A_wo, B_w_gate, B_w_up, B_w_down)
    return out.reshape(B, S, D)
```

```python
import math

import jax
import jax.numpy as jnp
from jax import lax
import jax.experimental.pallas as pl
import jax.experimental.pallas.tpu as pltpu

F32 = jnp.float32
BF16 = jnp.bfloat16

NUM_HEADS = 32
LN_EPS = 1e-5
DEN_EPS = 1e-6
LOG2E = math.log2(math.e)
LANES = 128

KV_SUB = 128
KV_UNROLL = 4
Q_SUB = 256
Q_UNROLL = 2
FFN_CHUNK = 512

_NN = (((1,), (0,)), ((), ()))
_NT = (((1,), (1,)), ((), ()))


def _dot(a, b, dims=_NN):
    return lax.dot_general(a, b, dims, preferred_element_type=F32)


def _iota(shape, dim):
    return lax.broadcasted_iota(jnp.int32, shape, dim)


def _idiv(v, n):
    return ((v.astype(F32) + 0.5) * (1.0 / n)).astype(jnp.int32)


def _layernorm(x):
    m = jnp.mean(x, axis=-1, keepdims=True)
    d = x - m
    var = jnp.mean(d * d, axis=-1, keepdims=True)
    return d * lax.rsqrt(var + LN_EPS)


def _gelu(x):
    c = math.sqrt(2.0 / math.pi)
    inner = x * (c + (c * 0.044715) * (x * x))
    return (0.5 * x) * (1.0 + jnp.tanh(inner))


def _per_head(v, op):
    v = op(v, pltpu.roll(v, 4, 0))
    return op(v, pltpu.roll(v, 2, 0))


def _dual_exp(p):
    rows, t = p.shape
    p3 = p.reshape(rows // 8, 8, t)
    mx = _per_head(jnp.max(p3, axis=0), jnp.maximum)
    mn = _per_head(jnp.min(p3, axis=0), jnp.minimum)
    e_pos = jnp.exp2(p3 - mx[None])
    e_neg = jnp.exp2(mn[None] - p3)
    s_pos = _per_head(jnp.sum(e_pos, axis=0), jnp.add)
    s_neg = _per_head(jnp.sum(e_neg, axis=0), jnp.add)
    return e_pos, e_neg, s_pos, s_neg


def _scale(e, r):
    n, _, t = e.shape
    return (e * r[None]).reshape(n * 8, t)


def _feature_tile(units):
    rows = sum(u.shape[0] for u in units)
    pad = jnp.zeros((LANES - rows, units[0].shape[1]), F32)
    return jnp.concatenate(list(units) + [pad], axis=0).astype(BF16)


def _kernel(x_hbm, wqkv_hbm, wphi_hbm, wo_hbm, wg_hbm, wu_hbm, wd_hbm, out_hbm,
            x_v, xn_v, wqkv_v, wt_v, wo_v, wg_v, wu_v, wd_v, out_v,
            wphi_v, phi_v, kv_acc, z_acc, kv_v, x_sem, w_sem, o_sem):
    S, D = x_v.shape
    F = wg_v.shape[1]
    Dh = D // NUM_HEADS
    NP = NUM_HEADS // 2
    PR = 2 * Dh
    NU = 2 * NP
    NT = -(-NU // 3)
    n1 = S // (KV_SUB * KV_UNROLL)
    n2 = S // (Q_SUB * Q_UNROLL)

    def tile_units(j):
        return list(range(3 * j, min(3 * j + 3, NU)))

    def tile_rows(j):
        us = tile_units(j)
        return (us[0] // 2) * PR, (us[-1] // 2 + 1) * PR

    def x_copy(i):
        rows = pl.ds(i * KV_SUB, KV_SUB)
        return pltpu.make_async_copy(x_hbm.at[rows], x_v.at[rows], x_sem.at[i])

    def wqkv_copy(i):
        cols = pl.ds(i * D, D)
        return pltpu.make_async_copy(wqkv_hbm.at[:, cols], wqkv_v.at[i], w_sem.at[i])

    wphi_copy = pltpu.make_async_copy(wphi_hbm, wphi_v, w_sem.at[3])
    late_copies = [
        wqkv_copy(0),
        pltpu.make_async_copy(wo_hbm, wo_v, w_sem.at[4]),
        pltpu.make_async_copy(wg_hbm, wg_v, w_sem.at[5]),
        pltpu.make_async_copy(wu_hbm, wu_v, w_sem.at[6]),
        pltpu.make_async_copy(wd_hbm, wd_v, w_sem.at[7]),
    ]

    def out_copy(i):
        rows = pl.ds(pl.multiple_of(i * Q_SUB, Q_SUB), Q_SUB)
        return pltpu.make_async_copy(out_v.at[rows], out_hbm.at[rows], o_sem.at[i])

    wphi_copy.start()
    x_copy(0).start()
    wqkv_copy(1).start()
    wqkv_copy(2).start()

    phi_v[...] = jnp.zeros(phi_v.shape, F32)
    kv_acc[...] = jnp.zeros(kv_acc.shape, F32)
    z_acc[...] = jnp.zeros(z_acc.shape, F32)
    wphi_copy.wait()
    for d in range(Dh):
        phi_v[pl.ds(d, NUM_HEADS, stride=Dh), 0:Dh] = wphi_v[d].astype(F32).T
    r = _iota((4 * PR, LANES), 0)
    c = _iota((4 * PR, LANES), 1)
    r_pair = _idiv(r, PR)
    pick_feature = (((r - r_pair * PR) >> 1) == c).astype(BF16)
    r_head = 2 * r_pair + (r & 1)
    phi_t = []
    for j in range(D // LANES):
        full = _dot(pick_feature, phi_v[j * LANES:(j + 1) * LANES, :].astype(BF16), _NT)
        own_head = (r_head + 6 * j) == _idiv(c + j * LANES, Dh)
        phi_t.append(jnp.where(own_head, full, 0.0).astype(BF16))

    def fold(i):
        pieces, tail = [], None
        for j in range(D // LANES):
            part = _dot(phi_t[j], wqkv_v[i, :, j * LANES:(j + 1) * LANES], _NT)
            pieces.append(part[:PR] if tail is None else part[:PR] + tail)
            pieces.append(part[PR:3 * PR])
            tail = part[3 * PR:]
        pieces.append(tail)
        wt_v[i] = (jnp.concatenate(pieces, axis=0) * LOG2E).astype(BF16)

    def norm_tile(i):
        rows = pl.ds(pl.multiple_of(i * KV_SUB, KV_SUB), KV_SUB)
        xn = _layernorm(x_v[rows, :].astype(F32)).astype(BF16)
        xn_v[rows, :] = xn
        return xn

    x_copy(0).wait()
    norm_tile(0)
    wqkv_copy(1).wait()
    for i in range(1, KV_UNROLL + 1):
        x_copy(i).start()
    fold(1)
    wqkv_copy(2).wait()
    for i in range(KV_UNROLL + 1, n1 * KV_UNROLL):
        x_copy(i).start()
    wt_v[2] = wqkv_v[2].T

    def kv_step(t, carry):
        first = t * KV_UNROLL
        for s in range(1, KV_UNROLL):
            x_copy(first + s).wait()

        @pl.when(t + 1 < n1)
        def _():
            x_copy(first + KV_UNROLL).wait()

        @pl.when(t == 1)
        def _():
            for cp in late_copies:
                cp.start()

        units, tiles, vts = [], [], []
        xn = xn_v[pl.ds(pl.multiple_of(first * KV_SUB, KV_SUB), KV_SUB), :]
        for s in range(KV_UNROLL):
            pk = _dot(wt_v[1], xn, _NT)
            us = []
            for p in range(NP):
                e_pos, e_neg, s_pos, s_neg = _dual_exp(pk[p * PR:(p + 1) * PR])
                inv = 1.0 / (s_pos * s_neg)
                us += [_scale(e_pos, s_neg * inv), _scale(e_neg, s_pos * inv)]
            units.append(us)
            tiles.append([_feature_tile([us[u] for u in tile_units(j)]) for j in range(NT)])
            if s + 1 < KV_UNROLL:
                xn_next = norm_tile(first + s + 1)
            else:
                xn_next = norm_tile(jnp.minimum(t + 1, n1 - 1) * KV_UNROLL)
            vts.append(_dot(wt_v[2], xn, _NT))
            xn = xn_next

        accs = [kv_acc[j, 0:tile_rows(j)[1] - tile_rows(j)[0], :] for j in range(NT)]
        for s in range(KV_UNROLL):
            for j in range(NT):
                lo, hi = tile_rows(j)
                accs[j] = accs[j] + _dot(vts[s][lo:hi].astype(BF16), tiles[s][j], _NT)
        for j in range(NT):
            kv_acc[j, 0:accs[j].shape[0], :] = accs[j]
        for u in range(NU):
            z = z_acc[u]
            for s in range(KV_UNROLL):
                z = z + units[s][u]
            z_acc[u] = z
        return carry

    lax.fori_loop(0, n1, kv_step, 0)
    for cp in late_copies:
        cp.wait()

    fold(0)
    r = _iota((2 * PR, LANES), 0)
    c = _iota((2 * PR, LANES), 1)
    for j in range(NT):
        row_head = _idiv(r + tile_rows(j)[0], Dh)
        col_head = 2 * ((_idiv(c, PR) + 3 * j) >> 1) + (c & 1)
        kv_v[j] = jnp.where(row_head == col_head, kv_acc[j], 0.0).astype(BF16)
    for u in range(NU):
        z_acc[u] = jnp.broadcast_to(jnp.sum(z_acc[u], axis=1, keepdims=True), (PR, LANES))

    def query_features(pq):
        units = []
        for p in range(NP):
            e_pos, e_neg, s_pos, s_neg = _dual_exp(pq[p * PR:(p + 1) * PR])

            def dot_z(e, u):
                z = jnp.concatenate([z_acc[u]] * (Q_SUB // LANES), axis=1).reshape(e.shape)
                return jnp.sum(e * z, axis=0)

            den = _per_head(dot_z(e_pos, 2 * p) * s_neg + dot_z(e_neg, 2 * p + 1) * s_pos, jnp.add)
            inv = 1.0 / (den + DEN_EPS * (s_pos * s_neg))
            units += [_scale(e_pos, s_neg * inv), _scale(e_neg, s_pos * inv)]
        return units

    def attend(units):
        outs = [None] * NP
        for j in range(NT):
            lo, hi = tile_rows(j)
            res = _dot(kv_v[j, 0:hi - lo, :], _feature_tile([units[u] for u in tile_units(j)]))
            for i in range((hi - lo) // PR):
                p = lo // PR + i
                piece = res[i * PR:(i + 1) * PR]
                outs[p] = piece if outs[p] is None else outs[p] + piece
        return jnp.concatenate(outs, axis=0).astype(BF16).T

    def q_step(t, carry):
        subs = [t * Q_UNROLL + s for s in range(Q_UNROLL)]
        rows = [pl.ds(pl.multiple_of(i * Q_SUB, Q_SUB), Q_SUB) for i in subs]
        feats = [query_features(_dot(wt_v[0], xn_v[r, :], _NT)) for r in rows]
        attn = [attend(f) for f in feats]
        hs = [x_v[r, :].astype(F32) + _dot(o, wo_v[...]) for r, o in zip(rows, attn)]
        for i, r, h in zip(subs, rows, hs):
            hn = _layernorm(h).astype(BF16)
            acc = h
            for c in range(F // FFN_CHUNK):
                cols = slice(c * FFN_CHUNK, (c + 1) * FFN_CHUNK)
                act = _gelu(_dot(hn, wg_v[:, cols])) * _dot(hn, wu_v[:, cols])
                acc = acc + _dot(act.astype(BF16), wd_v[cols, :])
            out_v[r, :] = acc.astype(out_v.dtype)
            out_copy(i).start()
        return carry

    lax.fori_loop(0, n2, q_step, 0)
    for i in range(n2 * Q_UNROLL):
        out_copy(i).wait()


@jax.jit
def pallas_sequential_preLN__linear_kernel_hedgehog__geglu_ffn__prompt_kernel(
    A_x: jax.Array,
    A_wqkv: jax.Array,
    A_w_phi: jax.Array,
    A_wo: jax.Array,
    B_x: jax.Array,
    B_w_gate: jax.Array,
    B_w_up: jax.Array,
    B_w_down: jax.Array,
):
    del B_x
    B, S, D = A_x.shape
    F = B_w_gate.shape[1]
    Dh = D // NUM_HEADS
    NT = -(-NUM_HEADS // 3)
    assert B == 1 and Dh == 20 and KV_SUB == LANES
    assert S % (KV_SUB * KV_UNROLL) == 0 and S // (KV_SUB * KV_UNROLL) >= 2
    assert S % (Q_SUB * Q_UNROLL) == 0 and F % FFN_CHUNK == 0
    hbm = pl.BlockSpec(memory_space=pl.ANY)
    out = pl.pallas_call(
        _kernel,
        out_shape=jax.ShapeDtypeStruct((S, D), A_x.dtype),
        in_specs=[hbm] * 7,
        out_specs=hbm,
        scratch_shapes=[
            pltpu.VMEM((S, D), A_x.dtype),
            pltpu.VMEM((S, D), BF16),
            pltpu.VMEM((3, D, D), A_wqkv.dtype),
            pltpu.VMEM((3, D, D), BF16),
            pltpu.VMEM((D, D), A_wo.dtype),
            pltpu.VMEM((D, F), B_w_gate.dtype),
            pltpu.VMEM((D, F), B_w_up.dtype),
            pltpu.VMEM((F, D), B_w_down.dtype),
            pltpu.VMEM((S, D), A_x.dtype),
            pltpu.VMEM((Dh, Dh, NUM_HEADS), A_w_phi.dtype),
            pltpu.VMEM((D, LANES), F32),
            pltpu.VMEM((NT, 4 * Dh, LANES), F32),
            pltpu.VMEM((NUM_HEADS, 2 * Dh, LANES), F32),
            pltpu.VMEM((NT, 4 * Dh, LANES), BF16),
            pltpu.SemaphoreType.DMA((S // KV_SUB,)),
            pltpu.SemaphoreType.DMA((8,)),
            pltpu.SemaphoreType.DMA((S // Q_SUB,)),
        ],
        compiler_params=pltpu.CompilerParams(vmem_limit_bytes=100 * 1024 * 1024),
    )(A_x.reshape(S, D), A_wqkv, A_w_phi.transpose(1, 2, 0), A_wo, B_w_gate, B_w_up, B_w_down)
    return out.reshape(B, S, D)
```

```python
import math

import jax
import jax.numpy as jnp
from jax import lax
import jax.experimental.pallas as pl
import jax.experimental.pallas.tpu as pltpu

F32 = jnp.float32
BF16 = jnp.bfloat16

NUM_HEADS = 32
LN_EPS = 1e-5
DEN_EPS = 1e-6
LOG2E = math.log2(math.e)
LANES = 128

KV_SUB = 128
KV_UNROLL = 4
Q_SUB = 256
Q_UNROLL = 2
FFN_CHUNK = 512

_NN = (((1,), (0,)), ((), ()))
_NT = (((1,), (1,)), ((), ()))


def _dot(a, b, dims=_NN):
    return lax.dot_general(a, b, dims, preferred_element_type=F32)


def _iota(shape, dim):
    return lax.broadcasted_iota(jnp.int32, shape, dim)


def _idiv(v, n):
    return ((v.astype(F32) + 0.5) * (1.0 / n)).astype(jnp.int32)


def _layernorm(x):
    m = jnp.mean(x, axis=-1, keepdims=True)
    d = x - m
    var = jnp.mean(d * d, axis=-1, keepdims=True)
    return d * lax.rsqrt(var + LN_EPS)


def _gelu(x):
    c = math.sqrt(2.0 / math.pi)
    inner = x * (c + (c * 0.044715) * (x * x))
    return (0.5 * x) * (1.0 + jnp.tanh(inner))


def _per_head(v, op):
    v = op(v, pltpu.roll(v, 4, 0))
    return op(v, pltpu.roll(v, 2, 0))


def _dual_exp(p):
    rows, t = p.shape
    p3 = p.reshape(rows // 8, 8, t)
    mx = _per_head(jnp.max(p3, axis=0), jnp.maximum)
    mn = _per_head(jnp.min(p3, axis=0), jnp.minimum)
    e_pos = jnp.exp2(p3 - mx[None])
    e_neg = jnp.exp2(mn[None] - p3)
    s_pos = _per_head(jnp.sum(e_pos, axis=0), jnp.add)
    s_neg = _per_head(jnp.sum(e_neg, axis=0), jnp.add)
    return e_pos, e_neg, s_pos, s_neg


def _features(e_pos, e_neg, scale_pos, scale_neg):
    n, _, t = e_pos.shape
    return jnp.concatenate([(e_pos * scale_pos[None]).reshape(n * 8, t),
                            (e_neg * scale_neg[None]).reshape(n * 8, t)], axis=0)


def _kernel(x_hbm, wqkv_hbm, wphi_hbm, wo_hbm, wg_hbm, wu_hbm, wd_hbm, out_hbm,
            x_v, xn_v, wqkv_v, wt_v, wo_v, wg_v, wu_v, wd_v, out_v,
            wphi_v, phi_v, kv_acc, z_acc, x_sem, w_sem, o_sem):
    S, D = x_v.shape
    F = wg_v.shape[1]
    Dh = D // NUM_HEADS
    NP = NUM_HEADS // 2
    PR = 2 * Dh
    KV_TILE = KV_SUB * KV_UNROLL
    n1 = S // KV_TILE
    n2 = S // (Q_SUB * Q_UNROLL)

    def pair(p):
        return slice(p * PR, (p + 1) * PR)

    def x_copy(i, lo, hi):
        rows = pl.ds(lo, hi - lo)
        return pltpu.make_async_copy(x_hbm.at[rows], x_v.at[rows], x_sem.at[i])

    x_first = x_copy(0, 0, KV_SUB)
    x_step0 = x_copy(1, KV_SUB, KV_TILE + KV_SUB)
    x_rest = x_copy(2, KV_TILE + KV_SUB, S)

    def wqkv_copy(i):
        cols = pl.ds(i * D, D)
        return pltpu.make_async_copy(wqkv_hbm.at[:, cols], wqkv_v.at[i], w_sem.at[i])

    wphi_copy = pltpu.make_async_copy(wphi_hbm, wphi_v, w_sem.at[3])
    late_copies = [
        wqkv_copy(0),
        pltpu.make_async_copy(wo_hbm, wo_v, w_sem.at[4]),
        pltpu.make_async_copy(wg_hbm, wg_v, w_sem.at[5]),
        pltpu.make_async_copy(wu_hbm, wu_v, w_sem.at[6]),
        pltpu.make_async_copy(wd_hbm, wd_v, w_sem.at[7]),
    ]

    def out_copy(i):
        rows = pl.ds(pl.multiple_of(i * Q_SUB, Q_SUB), Q_SUB)
        return pltpu.make_async_copy(out_v.at[rows], out_hbm.at[rows], o_sem.at[i])

    wphi_copy.start()
    x_first.start()
    wqkv_copy(1).start()
    wqkv_copy(2).start()
    x_step0.start()

    phi_v[...] = jnp.zeros(phi_v.shape, F32)
    kv_acc[...] = jnp.zeros(kv_acc.shape, F32)
    z_acc[...] = jnp.zeros(z_acc.shape, F32)
    wphi_copy.wait()
    for d in range(Dh):
        phi_v[pl.ds(d, NUM_HEADS, stride=Dh), 0:Dh] = wphi_v[d].astype(F32).T
    r = _iota((4 * PR, LANES), 0)
    c = _iota((4 * PR, LANES), 1)
    r_pair = _idiv(r, PR)
    pick_feature = (((r - r_pair * PR) >> 1) == c).astype(BF16)
    r_head = 2 * r_pair + (r & 1)
    phi_t = []
    for j in range(D // LANES):
        full = _dot(pick_feature, phi_v[j * LANES:(j + 1) * LANES, :].astype(BF16), _NT)
        own_head = (r_head + 6 * j) == _idiv(c + j * LANES, Dh)
        phi_t.append(jnp.where(own_head, full, 0.0).astype(BF16))

    def fold(i):
        pieces, tail = [], None
        for j in range(D // LANES):
            part = _dot(phi_t[j], wqkv_v[i, :, j * LANES:(j + 1) * LANES], _NT)
            pieces.append(part[:PR] if tail is None else part[:PR] + tail)
            pieces.append(part[PR:3 * PR])
            tail = part[3 * PR:]
        pieces.append(tail)
        wt_v[i] = (jnp.concatenate(pieces, axis=0) * LOG2E).astype(BF16)

    def norm_tile(i):
        rows = pl.ds(pl.multiple_of(i * KV_SUB, KV_SUB), KV_SUB)
        xn = _layernorm(x_v[rows, :].astype(F32)).astype(BF16)
        xn_v[rows, :] = xn
        return xn

    x_first.wait()
    norm_tile(0)
    wqkv_copy(1).wait()
    fold(1)
    wqkv_copy(2).wait()
    wt_v[2] = wqkv_v[2].T
    x_step0.wait()
    x_rest.start()

    def kv_step(t, carry):
        @pl.when(t == 0)
        def _():
            for cp in late_copies:
                cp.start()

        @pl.when(t == 1)
        def _():
            x_rest.wait()

        first = t * KV_UNROLL
        phis, vts = [], []
        xn = xn_v[pl.ds(pl.multiple_of(first * KV_SUB, KV_SUB), KV_SUB), :]
        for s in range(KV_UNROLL):
            pk = _dot(wt_v[1], xn, _NT)
            phi = []
            for p in range(NP):
                e_pos, e_neg, s_pos, s_neg = _dual_exp(pk[pair(p)])
                inv = 1.0 / (s_pos * s_neg)
                phi.append(_features(e_pos, e_neg, s_neg * inv, s_pos * inv))
            phis.append(phi)
            if s + 1 < KV_UNROLL:
                xn_next = norm_tile(first + s + 1)
            else:
                xn_next = norm_tile(jnp.minimum(t + 1, n1 - 1) * KV_UNROLL)
            vts.append(_dot(wt_v[2], xn, _NT))
            xn = xn_next

        for p in range(NP):
            vt = jnp.concatenate([v[pair(p)] for v in vts], axis=1)
            phi = jnp.concatenate([f[p] for f in phis], axis=1)
            kv_acc[p] += _dot(vt, phi, _NT)
        for p in range(NP):
            z = phis[0][p]
            for f in phis[1:]:
                z = z + f[p]
            z_acc[p] += z
        return carry

    lax.fori_loop(0, n1, kv_step, 0)
    for cp in late_copies:
        cp.wait()

    fold(0)
    own_head = _idiv(_iota((PR, 2 * PR), 0), Dh) == (_iota((PR, 2 * PR), 1) & 1)
    for p in range(NP):
        kv_acc[p] = jnp.where(own_head, kv_acc[p], 0.0)
        z_acc[p] = jnp.broadcast_to(jnp.sum(z_acc[p], axis=1, keepdims=True), (2 * PR, LANES))

    def query_features(pq):
        phi = []
        for p in range(NP):
            e_pos, e_neg, s_pos, s_neg = _dual_exp(pq[pair(p)])

            def dot_z(e, rows):
                z = jnp.concatenate([z_acc[p, rows, :]] * (Q_SUB // LANES), axis=1)
                return jnp.sum(e * z.reshape(e.shape), axis=0)

            den = _per_head(dot_z(e_pos, pair(0)) * s_neg + dot_z(e_neg, pair(1)) * s_pos, jnp.add)
            inv = 1.0 / (den + DEN_EPS * (s_pos * s_neg))
            phi.append(_features(e_pos, e_neg, s_neg * inv, s_pos * inv))
        return phi

    def attend(phi):
        ot = jnp.concatenate([_dot(kv_acc[p], phi[p]) for p in range(NP)], axis=0)
        return ot.astype(BF16).T

    def q_step(t, carry):
        subs = [t * Q_UNROLL + s for s in range(Q_UNROLL)]
        rows = [pl.ds(pl.multiple_of(i * Q_SUB, Q_SUB), Q_SUB) for i in subs]
        feats = [query_features(_dot(wt_v[0], xn_v[r, :], _NT)) for r in rows]
        attn = [attend(f) for f in feats]
        hs = [x_v[r, :].astype(F32) + _dot(o, wo_v[...]) for r, o in zip(rows, attn)]
        for i, r, h in zip(subs, rows, hs):
            hn = _layernorm(h).astype(BF16)
            acc = h
            for c in range(F // FFN_CHUNK):
                cols = slice(c * FFN_CHUNK, (c + 1) * FFN_CHUNK)
                act = _gelu(_dot(hn, wg_v[:, cols])) * _dot(hn, wu_v[:, cols])
                acc = acc + _dot(act.astype(BF16), wd_v[cols, :])
            out_v[r, :] = acc.astype(out_v.dtype)
            out_copy(i).start()
        return carry

    lax.fori_loop(0, n2, q_step, 0)
    for i in range(n2 * Q_UNROLL):
        out_copy(i).wait()


@jax.jit
def pallas_sequential_preLN__linear_kernel_hedgehog__geglu_ffn__prompt_kernel(
    A_x: jax.Array,
    A_wqkv: jax.Array,
    A_w_phi: jax.Array,
    A_wo: jax.Array,
    B_x: jax.Array,
    B_w_gate: jax.Array,
    B_w_up: jax.Array,
    B_w_down: jax.Array,
):
    del B_x
    B, S, D = A_x.shape
    F = B_w_gate.shape[1]
    Dh = D // NUM_HEADS
    NP = NUM_HEADS // 2
    assert B == 1 and Dh == 20 and KV_SUB == LANES
    assert S % (KV_SUB * KV_UNROLL) == 0 and S // (KV_SUB * KV_UNROLL) >= 2
    assert S % (Q_SUB * Q_UNROLL) == 0 and F % FFN_CHUNK == 0
    hbm = pl.BlockSpec(memory_space=pl.ANY)
    out = pl.pallas_call(
        _kernel,
        out_shape=jax.ShapeDtypeStruct((S, D), A_x.dtype),
        in_specs=[hbm] * 7,
        out_specs=hbm,
        scratch_shapes=[
            pltpu.VMEM((S, D), A_x.dtype),
            pltpu.VMEM((S, D), BF16),
            pltpu.VMEM((3, D, D), A_wqkv.dtype),
            pltpu.VMEM((3, D, D), BF16),
            pltpu.VMEM((D, D), A_wo.dtype),
            pltpu.VMEM((D, F), B_w_gate.dtype),
            pltpu.VMEM((D, F), B_w_up.dtype),
            pltpu.VMEM((F, D), B_w_down.dtype),
            pltpu.VMEM((S, D), A_x.dtype),
            pltpu.VMEM((Dh, Dh, NUM_HEADS), A_w_phi.dtype),
            pltpu.VMEM((D, LANES), F32),
            pltpu.VMEM((NP, 2 * Dh, 4 * Dh), F32),
            pltpu.VMEM((NP, 4 * Dh, LANES), F32),
            pltpu.SemaphoreType.DMA((3,)),
            pltpu.SemaphoreType.DMA((8,)),
            pltpu.SemaphoreType.DMA((S // Q_SUB,)),
        ],
        compiler_params=pltpu.CompilerParams(vmem_limit_bytes=100 * 1024 * 1024),
    )(A_x.reshape(S, D), A_wqkv, A_w_phi.transpose(1, 2, 0), A_wo, B_w_gate, B_w_up, B_w_down)
    return out.reshape(B, S, D)
```

```python
import math

import jax
import jax.numpy as jnp
from jax import lax
import jax.experimental.pallas as pl
import jax.experimental.pallas.tpu as pltpu

F32 = jnp.float32
BF16 = jnp.bfloat16

NUM_HEADS = 32
LN_EPS = 1e-5
DEN_EPS = 1e-6
LOG2E = math.log2(math.e)
LANES = 128

KV_SUB = 128
KV_HEAD = 2
KV_UNROLL = 7
Q_SUB = 256
Q_UNROLL = 2
FFN_CHUNK = 512

_NN = (((1,), (0,)), ((), ()))
_NT = (((1,), (1,)), ((), ()))


def _dot(a, b, dims=_NN):
    return lax.dot_general(a, b, dims, precision=lax.Precision.DEFAULT, preferred_element_type=F32)


def _iota(shape, dim):
    return lax.broadcasted_iota(jnp.int32, shape, dim)


def _idiv(v, n):
    return ((v.astype(F32) + 0.5) * (1.0 / n)).astype(jnp.int32)


def _layernorm(x):
    m = jnp.mean(x, axis=-1, keepdims=True)
    d = x - m
    var = jnp.mean(d * d, axis=-1, keepdims=True)
    return d * lax.rsqrt(var + LN_EPS)


def _gelu(x):
    c = math.sqrt(2.0 / math.pi)
    inner = x * (c + (c * 0.044715) * (x * x))
    return (0.5 * x) * (1.0 + jnp.tanh(inner))


def _per_head(v, op):
    v = op(v, pltpu.roll(v, 4, 0))
    return op(v, pltpu.roll(v, 2, 0))


def _dual_exp(p):
    rows, t = p.shape
    p3 = p.reshape(rows // 8, 8, t)
    mx = _per_head(jnp.max(p3, axis=0), jnp.maximum)
    mn = _per_head(jnp.min(p3, axis=0), jnp.minimum)
    e_pos = jnp.exp2(p3 - mx[None])
    e_neg = jnp.exp2(mn[None] - p3)
    s_pos = _per_head(jnp.sum(e_pos, axis=0), jnp.add)
    s_neg = _per_head(jnp.sum(e_neg, axis=0), jnp.add)
    return e_pos, e_neg, s_pos, s_neg


def _features(e_pos, e_neg, scale_pos, scale_neg):
    n, _, t = e_pos.shape
    return jnp.concatenate([(e_pos * scale_pos[None]).reshape(n * 8, t),
                            (e_neg * scale_neg[None]).reshape(n * 8, t)], axis=0)


def _kernel(x_hbm, wqkv_hbm, wphi_hbm, wo_hbm, wg_hbm, wu_hbm, wd_hbm, out_hbm,
            x_v, xn_v, wqkv_v, wt_v, wo_v, wg_v, wu_v, wd_v, out_v,
            wphi_v, phi_v, kv_acc, z_acc, x_sem, w_sem, o_sem):
    S, D = x_v.shape
    F = wg_v.shape[1]
    Dh = D // NUM_HEADS
    NP = NUM_HEADS // 2
    PR = 2 * Dh
    n1 = (S // KV_SUB - KV_HEAD) // KV_UNROLL
    n2 = S // (Q_SUB * Q_UNROLL)

    def pair(p):
        return slice(p * PR, (p + 1) * PR)

    def x_copy(i, lo, hi):
        rows = pl.ds(lo, hi - lo)
        return pltpu.make_async_copy(x_hbm.at[rows], x_v.at[rows], x_sem.at[i])

    x_head = x_copy(0, 0, (KV_HEAD + 1) * KV_SUB)
    x_step0 = x_copy(1, (KV_HEAD + 1) * KV_SUB, (KV_HEAD + 1 + KV_UNROLL) * KV_SUB)
    x_rest = x_copy(2, (KV_HEAD + 1 + KV_UNROLL) * KV_SUB, S)

    def wqkv_copy(i):
        cols = pl.ds(i * D, D)
        return pltpu.make_async_copy(wqkv_hbm.at[:, cols], wqkv_v.at[i], w_sem.at[i])

    wphi_copy = pltpu.make_async_copy(wphi_hbm, wphi_v, w_sem.at[3])
    late_copies = [
        wqkv_copy(0),
        pltpu.make_async_copy(wo_hbm, wo_v, w_sem.at[4]),
        pltpu.make_async_copy(wg_hbm, wg_v, w_sem.at[5]),
        pltpu.make_async_copy(wu_hbm, wu_v, w_sem.at[6]),
        pltpu.make_async_copy(wd_hbm, wd_v, w_sem.at[7]),
    ]

    def out_copy(i):
        rows = pl.ds(pl.multiple_of(i * Q_SUB, Q_SUB), Q_SUB)
        return pltpu.make_async_copy(out_v.at[rows], out_hbm.at[rows], o_sem.at[i])

    wphi_copy.start()
    wqkv_copy(1).start()
    x_head.start()
    wqkv_copy(2).start()
    x_step0.start()

    phi_v[...] = jnp.zeros(phi_v.shape, F32)
    kv_acc[...] = jnp.zeros(kv_acc.shape, F32)
    z_acc[...] = jnp.zeros(z_acc.shape, F32)
    wphi_copy.wait()
    for d in range(Dh):
        phi_v[pl.ds(d, NUM_HEADS, stride=Dh), 0:Dh] = wphi_v[d].astype(F32).T
    r = _iota((4 * PR, LANES), 0)
    c = _iota((4 * PR, LANES), 1)
    r_pair = _idiv(r, PR)
    pick_feature = (((r - r_pair * PR) >> 1) == c).astype(BF16)
    r_head = 2 * r_pair + (r & 1)
    phi_t = []
    for j in range(D // LANES):
        full = _dot(pick_feature, phi_v[j * LANES:(j + 1) * LANES, :].astype(BF16), _NT)
        own_head = (r_head + 6 * j) == _idiv(c + j * LANES, Dh)
        phi_t.append(jnp.where(own_head, full, 0.0).astype(BF16))

    def fold(i):
        pieces, tail = [], None
        for j in range(D // LANES):
            part = _dot(phi_t[j], wqkv_v[i, :, j * LANES:(j + 1) * LANES], _NT)
            pieces.append(part[:PR] if tail is None else part[:PR] + tail)
            pieces.append(part[PR:3 * PR])
            tail = part[3 * PR:]
        pieces.append(tail)
        wt_v[i] = (jnp.concatenate(pieces, axis=0) * LOG2E).astype(BF16)

    def norm_tile(i):
        rows = pl.ds(pl.multiple_of(i * KV_SUB, KV_SUB), KV_SUB)
        xn = _layernorm(x_v[rows, :].astype(F32)).astype(BF16)
        xn_v[rows, :] = xn
        return xn

    def key_features(pk):
        phi = []
        for p in range(NP):
            e_pos, e_neg, s_pos, s_neg = _dual_exp(pk[pair(p)])
            inv = 1.0 / (s_pos * s_neg)
            phi.append(_features(e_pos, e_neg, s_neg * inv, s_pos * inv))
        return phi

    def accumulate(vts, phis):
        for p in range(NP):
            vt = jnp.concatenate([v[pair(p)] for v in vts], axis=1)
            phi = jnp.concatenate([f[p] for f in phis], axis=1)
            kv_acc[p] += _dot(vt, phi, _NT)
        for p in range(NP):
            z = phis[0][p]
            for f in phis[1:]:
                z = z + f[p]
            z_acc[p] += z

    wqkv_copy(1).wait()
    fold(1)
    x_head.wait()
    for i in range(KV_HEAD + 1):
        norm_tile(i)
    xn = xn_v[0:KV_HEAD * KV_SUB, :]
    pk = _dot(wt_v[1], xn, _NT)
    phis = [key_features(pk[:, i * KV_SUB:(i + 1) * KV_SUB]) for i in range(KV_HEAD)]
    wqkv_copy(2).wait()
    wt_v[2] = wqkv_v[2].T
    accumulate([_dot(wt_v[2], xn, _NT)], phis)
    x_step0.wait()
    x_rest.start()

    def kv_step(t, carry):
        @pl.when(t == 0)
        def _():
            for cp in late_copies:
                cp.start()

        @pl.when(t == 1)
        def _():
            x_rest.wait()

        first = KV_HEAD + t * KV_UNROLL
        xns = [xn_v[pl.ds(pl.multiple_of(first * KV_SUB, KV_SUB), KV_SUB), :]]
        xns += [norm_tile(first + s) for s in range(1, KV_UNROLL)]
        norm_tile(KV_HEAD + jnp.minimum(t + 1, n1 - 1) * KV_UNROLL)
        phis, vts = [], []
        for s in range(KV_UNROLL):
            phis.append(key_features(_dot(wt_v[1], xns[s], _NT)))
            if s % 2 == 0:
                vts.append(_dot(wt_v[2], jnp.concatenate(xns[s:s + 2], axis=0), _NT))
        accumulate(vts, phis)
        return carry

    lax.fori_loop(0, n1, kv_step, 0)
    for cp in late_copies:
        cp.wait()

    fold(0)
    own_head = _idiv(_iota((PR, 2 * PR), 0), Dh) == (_iota((PR, 2 * PR), 1) & 1)
    for p in range(NP):
        kv_acc[p] = jnp.where(own_head, kv_acc[p], 0.0)
        z_acc[p] = jnp.broadcast_to(jnp.sum(z_acc[p], axis=1, keepdims=True), (2 * PR, LANES))

    def query_features(pq):
        phi = []
        for p in range(NP):
            e_pos, e_neg, s_pos, s_neg = _dual_exp(pq[pair(p)])

            def dot_z(e, rows):
                z = jnp.concatenate([z_acc[p, rows, :]] * (Q_SUB // LANES), axis=1)
                return jnp.sum(e * z.reshape(e.shape), axis=0)

            den = _per_head(dot_z(e_pos, pair(0)) * s_neg + dot_z(e_neg, pair(1)) * s_pos, jnp.add)
            inv = 1.0 / (den + DEN_EPS * (s_pos * s_neg))
            phi.append(_features(e_pos, e_neg, s_neg * inv, s_pos * inv))
        return phi

    def attend(phi):
        ot = jnp.concatenate([_dot(kv_acc[p], phi[p]) for p in range(NP)], axis=0)
        return ot.astype(BF16).T

    def q_step(t, carry):
        subs = [t * Q_UNROLL + s for s in range(Q_UNROLL)]
        rows = [pl.ds(pl.multiple_of(i * Q_SUB, Q_SUB), Q_SUB) for i in subs]
        feats = [query_features(_dot(wt_v[0], xn_v[r, :], _NT)) for r in rows]
        attn = [attend(f) for f in feats]
        hs = [x_v[r, :].astype(F32) + _dot(o, wo_v[...]) for r, o in zip(rows, attn)]
        for i, r, h in zip(subs, rows, hs):
            hn = _layernorm(h).astype(BF16)
            acc = h
            for c in range(F // FFN_CHUNK):
                cols = slice(c * FFN_CHUNK, (c + 1) * FFN_CHUNK)
                act = _gelu(_dot(hn, wg_v[:, cols])) * _dot(hn, wu_v[:, cols])
                acc = acc + _dot(act.astype(BF16), wd_v[cols, :])
            out_v[r, :] = acc.astype(out_v.dtype)
            out_copy(i).start()
        return carry

    lax.fori_loop(0, n2, q_step, 0)
    for i in range(n2 * Q_UNROLL):
        out_copy(i).wait()


@jax.jit
def pallas_sequential_preLN__linear_kernel_hedgehog__geglu_ffn__prompt_kernel(
    A_x: jax.Array,
    A_wqkv: jax.Array,
    A_w_phi: jax.Array,
    A_wo: jax.Array,
    B_x: jax.Array,
    B_w_gate: jax.Array,
    B_w_up: jax.Array,
    B_w_down: jax.Array,
):
    del B_x
    B, S, D = A_x.shape
    F = B_w_gate.shape[1]
    Dh = D // NUM_HEADS
    NP = NUM_HEADS // 2
    assert B == 1 and Dh == 20 and KV_SUB == LANES
    assert S % KV_SUB == 0 and (S // KV_SUB - KV_HEAD) % KV_UNROLL == 0
    assert (S // KV_SUB - KV_HEAD) // KV_UNROLL >= 2
    assert S % (Q_SUB * Q_UNROLL) == 0 and F % FFN_CHUNK == 0
    hbm = pl.BlockSpec(memory_space=pl.ANY)
    out = pl.pallas_call(
        _kernel,
        out_shape=jax.ShapeDtypeStruct((S, D), A_x.dtype),
        in_specs=[hbm] * 7,
        out_specs=hbm,
        scratch_shapes=[
            pltpu.VMEM((S, D), A_x.dtype),
            pltpu.VMEM((S, D), BF16),
            pltpu.VMEM((3, D, D), A_wqkv.dtype),
            pltpu.VMEM((3, D, D), BF16),
            pltpu.VMEM((D, D), A_wo.dtype),
            pltpu.VMEM((D, F), B_w_gate.dtype),
            pltpu.VMEM((D, F), B_w_up.dtype),
            pltpu.VMEM((F, D), B_w_down.dtype),
            pltpu.VMEM((S, D), A_x.dtype),
            pltpu.VMEM((Dh, Dh, NUM_HEADS), A_w_phi.dtype),
            pltpu.VMEM((D + NUM_HEADS, LANES), F32),
            pltpu.VMEM((NP, 2 * Dh, 4 * Dh), F32),
            pltpu.VMEM((NP, 4 * Dh, LANES), F32),
            pltpu.SemaphoreType.DMA((3,)),
            pltpu.SemaphoreType.DMA((8,)),
            pltpu.SemaphoreType.DMA((S // Q_SUB,)),
        ],
        compiler_params=pltpu.CompilerParams(vmem_limit_bytes=100 * 1024 * 1024),
    )(A_x.reshape(S, D), A_wqkv, A_w_phi.transpose(1, 2, 0), A_wo, B_w_gate, B_w_up, B_w_down)
    return out.reshape(B, S, D)
```

```python
import math

import jax
import jax.numpy as jnp
from jax import lax
import jax.experimental.pallas as pl
import jax.experimental.pallas.tpu as pltpu

F32 = jnp.float32
BF16 = jnp.bfloat16

NUM_HEADS = 32
LN_EPS = 1e-5
DEN_EPS = 1e-6
LOG2E = math.log2(math.e)
LANES = 128

KV_SUB = 128
KV_HEAD = 2
KV_UNROLL = 7
Q_SUB = 256
Q_UNROLL = 2
FFN_CHUNK = 512

_NN = (((1,), (0,)), ((), ()))
_NT = (((1,), (1,)), ((), ()))


def _dot(a, b, dims=_NN):
    return lax.dot_general(a, b, dims, precision=lax.Precision.DEFAULT, preferred_element_type=F32)


def _iota(shape, dim):
    return lax.broadcasted_iota(jnp.int32, shape, dim)


def _idiv(v, n):
    return ((v.astype(F32) + 0.5) * (1.0 / n)).astype(jnp.int32)


def _layernorm(x):
    m = jnp.mean(x, axis=-1, keepdims=True)
    d = x - m
    var = jnp.mean(d * d, axis=-1, keepdims=True)
    return d * lax.rsqrt(var + LN_EPS)


def _gelu(x):
    c = math.sqrt(2.0 / math.pi)
    inner = x * (c + (c * 0.044715) * (x * x))
    return (0.5 * x) * (1.0 + jnp.tanh(inner))


def _per_head(v, op):
    v = op(v, pltpu.roll(v, 4, 0))
    return op(v, pltpu.roll(v, 2, 0))


def _dual_exp(p):
    rows, t = p.shape
    p3 = p.reshape(rows // 8, 8, t)
    mx = _per_head(jnp.max(p3, axis=0), jnp.maximum)
    mn = _per_head(jnp.min(p3, axis=0), jnp.minimum)
    e_pos = jnp.exp2(p3 - mx[None])
    e_neg = jnp.exp2(mn[None] - p3)
    s_pos = _per_head(jnp.sum(e_pos, axis=0), jnp.add)
    s_neg = _per_head(jnp.sum(e_neg, axis=0), jnp.add)
    return e_pos, e_neg, s_pos, s_neg


def _features(e_pos, e_neg, scale_pos, scale_neg):
    n, _, t = e_pos.shape
    return jnp.concatenate([(e_pos * scale_pos[None]).reshape(n * 8, t),
                            (e_neg * scale_neg[None]).reshape(n * 8, t)], axis=0)


def _kernel(x_hbm, wqkv_hbm, wphi_hbm, wo_hbm, wg_hbm, wu_hbm, wd_hbm, out_hbm,
            x_v, xn_v, wqkv_v, wt_v, wo_v, wg_v, wu_v, wd_v, out_v,
            wphi_v, phi_v, kv_acc, z_acc, x_sem, w_sem, o_sem):
    S, D = x_v.shape
    F = wg_v.shape[1]
    Dh = D // NUM_HEADS
    NP = NUM_HEADS // 2
    PR = 2 * Dh
    n1 = (S // KV_SUB - KV_HEAD) // KV_UNROLL
    n2 = S // (Q_SUB * Q_UNROLL)

    def pair(p):
        return slice(p * PR, (p + 1) * PR)

    def x_copy(i, lo, hi):
        rows = pl.ds(lo, hi - lo)
        return pltpu.make_async_copy(x_hbm.at[rows], x_v.at[rows], x_sem.at[i])

    x_head = x_copy(0, 0, (KV_HEAD + 1) * KV_SUB)
    x_step0 = x_copy(1, (KV_HEAD + 1) * KV_SUB, (KV_HEAD + 1 + KV_UNROLL) * KV_SUB)
    x_rest = x_copy(2, (KV_HEAD + 1 + KV_UNROLL) * KV_SUB, S)

    def wqkv_copy(i):
        cols = pl.ds(i * D, D)
        return pltpu.make_async_copy(wqkv_hbm.at[:, cols], wqkv_v.at[i], w_sem.at[i])

    wphi_copy = pltpu.make_async_copy(wphi_hbm, wphi_v, w_sem.at[3])
    late_copies = [
        wqkv_copy(0),
        pltpu.make_async_copy(wo_hbm, wo_v, w_sem.at[4]),
        pltpu.make_async_copy(wg_hbm, wg_v, w_sem.at[5]),
        pltpu.make_async_copy(wu_hbm, wu_v, w_sem.at[6]),
        pltpu.make_async_copy(wd_hbm, wd_v, w_sem.at[7]),
    ]

    def out_copy(i):
        rows = pl.ds(pl.multiple_of(i * Q_SUB, Q_SUB), Q_SUB)
        return pltpu.make_async_copy(out_v.at[rows], out_hbm.at[rows], o_sem.at[i])

    wphi_copy.start()
    wqkv_copy(1).start()
    x_head.start()
    wqkv_copy(2).start()
    x_step0.start()

    phi_v[...] = jnp.zeros(phi_v.shape, F32)
    kv_acc[...] = jnp.zeros(kv_acc.shape, F32)
    z_acc[...] = jnp.zeros(z_acc.shape, F32)
    wphi_copy.wait()
    for d in range(Dh):
        phi_v[pl.ds(d, NUM_HEADS, stride=Dh), 0:Dh] = wphi_v[d].astype(F32).T
    r = _iota((4 * PR, LANES), 0)
    c = _iota((4 * PR, LANES), 1)
    r_pair = _idiv(r, PR)
    pick_feature = (((r - r_pair * PR) >> 1) == c).astype(BF16)
    r_head = 2 * r_pair + (r & 1)
    phi_t = []
    for j in range(D // LANES):
        full = _dot(pick_feature, phi_v[j * LANES:(j + 1) * LANES, :].astype(BF16), _NT)
        own_head = (r_head + 6 * j) == _idiv(c + j * LANES, Dh)
        phi_t.append(jnp.where(own_head, full, 0.0).astype(BF16))

    def fold(i):
        pieces, tail = [], None
        for j in range(D // LANES):
            part = _dot(phi_t[j], wqkv_v[i, :, j * LANES:(j + 1) * LANES], _NT)
            pieces.append(part[:PR] if tail is None else part[:PR] + tail)
            pieces.append(part[PR:3 * PR])
            tail = part[3 * PR:]
        pieces.append(tail)
        wt_v[i] = (jnp.concatenate(pieces, axis=0) * LOG2E).astype(BF16)

    def norm_tile(i):
        rows = pl.ds(pl.multiple_of(i * KV_SUB, KV_SUB), KV_SUB)
        xn = _layernorm(x_v[rows, :].astype(F32)).astype(BF16)
        xn_v[rows, :] = xn
        return xn

    def key_features(pk):
        phi = []
        for p in range(NP):
            e_pos, e_neg, s_pos, s_neg = _dual_exp(pk[pair(p)])
            inv = 1.0 / (s_pos * s_neg)
            phi.append(_features(e_pos, e_neg, s_neg * inv, s_pos * inv))
        return phi

    def accumulate(vts, phis):
        for p in range(NP):
            vt = jnp.concatenate([v[pair(p)] for v in vts], axis=1)
            phi = jnp.concatenate([f[p] for f in phis], axis=1)
            kv_acc[p] += _dot(vt, phi, _NT)
        for p in range(NP):
            z = phis[0][p]
            for f in phis[1:]:
                z = z + f[p]
            z_acc[p] += z

    wqkv_copy(1).wait()
    fold(1)
    x_head.wait()
    xns = [norm_tile(i) for i in range(KV_HEAD + 1)][:KV_HEAD]
    pks = [_dot(wt_v[1], xn, _NT) for xn in xns]
    wqkv_copy(2).wait()
    wt_v[2] = wqkv_v[2].T
    accumulate([_dot(wt_v[2], jnp.concatenate(xns, axis=0), _NT)], [key_features(pk) for pk in pks])
    x_step0.wait()
    x_rest.start()

    def kv_step(t, carry):
        @pl.when(t == 0)
        def _():
            for cp in late_copies:
                cp.start()

        @pl.when(t == 1)
        def _():
            x_rest.wait()

        first = KV_HEAD + t * KV_UNROLL
        xns = [xn_v[pl.ds(pl.multiple_of(first * KV_SUB, KV_SUB), KV_SUB), :]]
        xns += [norm_tile(first + s) for s in range(1, KV_UNROLL)]
        norm_tile(KV_HEAD + jnp.minimum(t + 1, n1 - 1) * KV_UNROLL)
        phis, vts = [], []
        for s in range(KV_UNROLL):
            phis.append(key_features(_dot(wt_v[1], xns[s], _NT)))
            if s % 2 == 0:
                vts.append(_dot(wt_v[2], jnp.concatenate(xns[s:s + 2], axis=0), _NT))
        accumulate(vts, phis)
        return carry

    lax.fori_loop(0, n1, kv_step, 0)
    for cp in late_copies:
        cp.wait()

    fold(0)
    own_head = _idiv(_iota((PR, 2 * PR), 0), Dh) == (_iota((PR, 2 * PR), 1) & 1)
    for p in range(NP):
        kv_acc[p] = jnp.where(own_head, kv_acc[p], 0.0)
        z_acc[p] = jnp.broadcast_to(jnp.sum(z_acc[p], axis=1, keepdims=True), (2 * PR, LANES))

    def query_features(pq):
        phi = []
        for p in range(NP):
            e_pos, e_neg, s_pos, s_neg = _dual_exp(pq[pair(p)])

            def dot_z(e, rows):
                z = jnp.concatenate([z_acc[p, rows, :]] * (Q_SUB // LANES), axis=1)
                return jnp.sum(e * z.reshape(e.shape), axis=0)

            den = _per_head(dot_z(e_pos, pair(0)) * s_neg + dot_z(e_neg, pair(1)) * s_pos, jnp.add)
            inv = 1.0 / (den + DEN_EPS * (s_pos * s_neg))
            phi.append(_features(e_pos, e_neg, s_neg * inv, s_pos * inv))
        return phi

    def attend(phi):
        ot = jnp.concatenate([_dot(kv_acc[p], phi[p]) for p in range(NP)], axis=0)
        return ot.astype(BF16).T

    def q_step(t, carry):
        subs = [t * Q_UNROLL + s for s in range(Q_UNROLL)]
        rows = [pl.ds(pl.multiple_of(i * Q_SUB, Q_SUB), Q_SUB) for i in subs]
        feats = [query_features(_dot(wt_v[0], xn_v[r, :], _NT)) for r in rows]
        attn = [attend(f) for f in feats]
        hs = [x_v[r, :].astype(F32) + _dot(o, wo_v[...]) for r, o in zip(rows, attn)]
        for i, r, h in zip(subs, rows, hs):
            hn = _layernorm(h).astype(BF16)
            acc = h
            for c in range(F // FFN_CHUNK):
                cols = slice(c * FFN_CHUNK, (c + 1) * FFN_CHUNK)
                act = _gelu(_dot(hn, wg_v[:, cols])) * _dot(hn, wu_v[:, cols])
                acc = acc + _dot(act.astype(BF16), wd_v[cols, :])
            out_v[r, :] = acc.astype(out_v.dtype)
            out_copy(i).start()
        return carry

    lax.fori_loop(0, n2, q_step, 0)
    for i in range(n2 * Q_UNROLL):
        out_copy(i).wait()


@jax.jit
def pallas_sequential_preLN__linear_kernel_hedgehog__geglu_ffn__prompt_kernel(
    A_x: jax.Array,
    A_wqkv: jax.Array,
    A_w_phi: jax.Array,
    A_wo: jax.Array,
    B_x: jax.Array,
    B_w_gate: jax.Array,
    B_w_up: jax.Array,
    B_w_down: jax.Array,
):
    del B_x
    B, S, D = A_x.shape
    F = B_w_gate.shape[1]
    Dh = D // NUM_HEADS
    NP = NUM_HEADS // 2
    assert B == 1 and Dh == 20 and KV_SUB == LANES
    assert S % KV_SUB == 0 and (S // KV_SUB - KV_HEAD) % KV_UNROLL == 0
    assert (S // KV_SUB - KV_HEAD) // KV_UNROLL >= 2
    assert S % (Q_SUB * Q_UNROLL) == 0 and F % FFN_CHUNK == 0
    hbm = pl.BlockSpec(memory_space=pl.ANY)
    out = pl.pallas_call(
        _kernel,
        out_shape=jax.ShapeDtypeStruct((S, D), A_x.dtype),
        in_specs=[hbm] * 7,
        out_specs=hbm,
        scratch_shapes=[
            pltpu.VMEM((S, D), A_x.dtype),
            pltpu.VMEM((S, D), BF16),
            pltpu.VMEM((3, D, D), A_wqkv.dtype),
            pltpu.VMEM((3, D, D), BF16),
            pltpu.VMEM((D, D), A_wo.dtype),
            pltpu.VMEM((D, F), B_w_gate.dtype),
            pltpu.VMEM((D, F), B_w_up.dtype),
            pltpu.VMEM((F, D), B_w_down.dtype),
            pltpu.VMEM((S, D), A_x.dtype),
            pltpu.VMEM((Dh, Dh, NUM_HEADS), A_w_phi.dtype),
            pltpu.VMEM((D + NUM_HEADS, LANES), F32),
            pltpu.VMEM((NP, 2 * Dh, 4 * Dh), F32),
            pltpu.VMEM((NP, 4 * Dh, LANES), F32),
            pltpu.SemaphoreType.DMA((3,)),
            pltpu.SemaphoreType.DMA((8,)),
            pltpu.SemaphoreType.DMA((S // Q_SUB,)),
        ],
        compiler_params=pltpu.CompilerParams(vmem_limit_bytes=100 * 1024 * 1024),
    )(A_x.reshape(S, D), A_wqkv, A_w_phi.transpose(1, 2, 0), A_wo, B_w_gate, B_w_up, B_w_down)
    return out.reshape(B, S, D)
```

```python
import math

import jax
import jax.numpy as jnp
from jax import lax
import jax.experimental.pallas as pl
import jax.experimental.pallas.tpu as pltpu

F32 = jnp.float32
BF16 = jnp.bfloat16

NUM_HEADS = 32
LN_EPS = 1e-5
DEN_EPS = 1e-6
LOG2E = math.log2(math.e)
LANES = 128

KV_SUB = 128
KV_HEAD = 2
KV_UNROLL = 7
Q_SUB = 256
Q_UNROLL = 2
FFN_CHUNK = 512
WK_LEAD = 2

_NN = (((1,), (0,)), ((), ()))
_NT = (((1,), (1,)), ((), ()))


def _dot(a, b, dims=_NN):
    return lax.dot_general(a, b, dims, precision=lax.Precision.DEFAULT, preferred_element_type=F32)


def _iota(shape, dim):
    return lax.broadcasted_iota(jnp.int32, shape, dim)


def _idiv(v, n):
    return ((v.astype(F32) + 0.5) * (1.0 / n)).astype(jnp.int32)


def _layernorm(x):
    m = jnp.mean(x, axis=-1, keepdims=True)
    d = x - m
    var = jnp.mean(d * d, axis=-1, keepdims=True)
    return d * lax.rsqrt(var + LN_EPS)


def _gelu(x):
    c = math.sqrt(2.0 / math.pi)
    inner = x * (c + (c * 0.044715) * (x * x))
    return (0.5 * x) * (1.0 + jnp.tanh(inner))


def _per_head(v, op):
    v = op(v, pltpu.roll(v, 4, 0))
    return op(v, pltpu.roll(v, 2, 0))


def _dual_exp(p):
    rows, t = p.shape
    p3 = p.reshape(rows // 8, 8, t)
    mx = _per_head(jnp.max(p3, axis=0), jnp.maximum)
    mn = _per_head(jnp.min(p3, axis=0), jnp.minimum)
    e_pos = jnp.exp2(p3 - mx[None])
    e_neg = jnp.exp2(mn[None] - p3)
    s_pos = _per_head(jnp.sum(e_pos, axis=0), jnp.add)
    s_neg = _per_head(jnp.sum(e_neg, axis=0), jnp.add)
    return e_pos, e_neg, s_pos, s_neg


def _features(e_pos, e_neg, scale_pos, scale_neg):
    n, _, t = e_pos.shape
    return jnp.concatenate([(e_pos * scale_pos[None]).reshape(n * 8, t),
                            (e_neg * scale_neg[None]).reshape(n * 8, t)], axis=0)


def _kernel(x_hbm, wqkv_hbm, wphi_hbm, wo_hbm, wg_hbm, wu_hbm, wd_hbm, out_hbm,
            x_v, xn_v, wqkv_v, wt_v, wo_v, wg_v, wu_v, wd_v, out_v,
            wphi_v, phi_v, kv_acc, z_acc, x_sem, w_sem, o_sem):
    S, D = x_v.shape
    F = wg_v.shape[1]
    Dh = D // NUM_HEADS
    NP = NUM_HEADS // 2
    PR = 2 * Dh
    n1 = (S // KV_SUB - KV_HEAD) // KV_UNROLL
    n2 = S // (Q_SUB * Q_UNROLL)

    def pair(p):
        return slice(p * PR, (p + 1) * PR)

    def x_copy(i, lo, hi):
        rows = pl.ds(lo, hi - lo)
        return pltpu.make_async_copy(x_hbm.at[rows], x_v.at[rows], x_sem.at[i])

    x_head = x_copy(0, 0, (KV_HEAD + 1) * KV_SUB)
    x_step0 = x_copy(1, (KV_HEAD + 1) * KV_SUB, (KV_HEAD + 1 + KV_UNROLL) * KV_SUB)
    x_rest = x_copy(2, (KV_HEAD + 1 + KV_UNROLL) * KV_SUB, S)

    def wqkv_copy(sem, i, lo=0, hi=D):
        return pltpu.make_async_copy(wqkv_hbm.at[:, pl.ds(i * D + lo, hi - lo)],
                                     wqkv_v.at[i, :, pl.ds(lo, hi - lo)], w_sem.at[sem])

    wk_lead = wqkv_copy(0, 1, 0, WK_LEAD * LANES)
    wk_rest = wqkv_copy(1, 1, WK_LEAD * LANES, D)
    wv_copy = wqkv_copy(2, 2)
    wphi_copy = pltpu.make_async_copy(wphi_hbm, wphi_v, w_sem.at[3])
    late_copies = [
        wqkv_copy(4, 0),
        pltpu.make_async_copy(wo_hbm, wo_v, w_sem.at[5]),
        pltpu.make_async_copy(wg_hbm, wg_v, w_sem.at[6]),
        pltpu.make_async_copy(wu_hbm, wu_v, w_sem.at[7]),
        pltpu.make_async_copy(wd_hbm, wd_v, w_sem.at[8]),
    ]

    def out_copy(i):
        rows = pl.ds(pl.multiple_of(i * Q_SUB, Q_SUB), Q_SUB)
        return pltpu.make_async_copy(out_v.at[rows], out_hbm.at[rows], o_sem.at[i])

    wphi_copy.start()
    wk_lead.start()
    wk_rest.start()
    x_head.start()
    wv_copy.start()
    x_step0.start()

    phi_v[...] = jnp.zeros(phi_v.shape, F32)
    kv_acc[...] = jnp.zeros(kv_acc.shape, F32)
    z_acc[...] = jnp.zeros(z_acc.shape, F32)
    wphi_copy.wait()
    for d in range(Dh):
        phi_v[pl.ds(d, NUM_HEADS, stride=Dh), 0:Dh] = wphi_v[d].astype(F32).T
    r = _iota((4 * PR, LANES), 0)
    c = _iota((4 * PR, LANES), 1)
    r_pair = _idiv(r, PR)
    pick_feature = (((r - r_pair * PR) >> 1) == c).astype(BF16)
    r_head = 2 * r_pair + (r & 1)
    phi_t = []
    for j in range(D // LANES):
        full = _dot(pick_feature, phi_v[j * LANES:(j + 1) * LANES, :].astype(BF16), _NT)
        own_head = (r_head + 6 * j) == _idiv(c + j * LANES, Dh)
        phi_t.append(jnp.where(own_head, full, 0.0).astype(BF16))

    def fold(i, rest=None):
        pieces, tail = [], None
        for j in range(D // LANES):
            if rest is not None and j == WK_LEAD:
                rest.wait()
            part = _dot(phi_t[j], wqkv_v[i, :, j * LANES:(j + 1) * LANES], _NT)
            pieces.append(part[:PR] if tail is None else part[:PR] + tail)
            pieces.append(part[PR:3 * PR])
            tail = part[3 * PR:]
        pieces.append(tail)
        wt_v[i] = (jnp.concatenate(pieces, axis=0) * LOG2E).astype(BF16)

    def norm_tile(i):
        rows = pl.ds(pl.multiple_of(i * KV_SUB, KV_SUB), KV_SUB)
        xn = _layernorm(x_v[rows, :].astype(F32)).astype(BF16)
        xn_v[rows, :] = xn
        return xn

    def key_features(pk):
        phi = []
        for p in range(NP):
            e_pos, e_neg, s_pos, s_neg = _dual_exp(pk[pair(p)])
            inv = 1.0 / (s_pos * s_neg)
            phi.append(_features(e_pos, e_neg, s_neg * inv, s_pos * inv))
        return phi

    def accumulate(vts, phis):
        for p in range(NP):
            vt = jnp.concatenate([v[pair(p)] for v in vts], axis=1)
            phi = jnp.concatenate([f[p] for f in phis], axis=1)
            kv_acc[p] += _dot(vt, phi, _NT)
        for p in range(NP):
            z = phis[0][p]
            for f in phis[1:]:
                z = z + f[p]
            z_acc[p] += z

    wk_lead.wait()
    fold(1, wk_rest)
    x_head.wait()
    xns = [norm_tile(i) for i in range(KV_HEAD + 1)][:KV_HEAD]
    pks = [_dot(wt_v[1], xn, _NT) for xn in xns]
    wv_copy.wait()
    wt_v[2] = wqkv_v[2].T
    accumulate([_dot(wt_v[2], jnp.concatenate(xns, axis=0), _NT)], [key_features(pk) for pk in pks])
    x_step0.wait()
    x_rest.start()

    def kv_step(t, carry):
        @pl.when(t == 0)
        def _():
            for cp in late_copies:
                cp.start()

        @pl.when(t == 1)
        def _():
            x_rest.wait()

        first = KV_HEAD + t * KV_UNROLL
        xns = [xn_v[pl.ds(pl.multiple_of(first * KV_SUB, KV_SUB), KV_SUB), :]]
        xns += [norm_tile(first + s) for s in range(1, KV_UNROLL)]
        norm_tile(KV_HEAD + jnp.minimum(t + 1, n1 - 1) * KV_UNROLL)
        phis, vts = [], []
        for s in range(KV_UNROLL):
            phis.append(key_features(_dot(wt_v[1], xns[s], _NT)))
            if s % 2 == 0:
                vts.append(_dot(wt_v[2], jnp.concatenate(xns[s:s + 2], axis=0), _NT))
        accumulate(vts, phis)
        return carry

    lax.fori_loop(0, n1, kv_step, 0)
    for cp in late_copies:
        cp.wait()

    fold(0)
    own_head = _idiv(_iota((PR, 2 * PR), 0), Dh) == (_iota((PR, 2 * PR), 1) & 1)
    for p in range(NP):
        kv_acc[p] = jnp.where(own_head, kv_acc[p], 0.0)
        z_acc[p] = jnp.broadcast_to(jnp.sum(z_acc[p], axis=1, keepdims=True), (2 * PR, LANES))

    def query_features(pq):
        phi = []
        for p in range(NP):
            e_pos, e_neg, s_pos, s_neg = _dual_exp(pq[pair(p)])

            def dot_z(e, rows):
                z = jnp.concatenate([z_acc[p, rows, :]] * (Q_SUB // LANES), axis=1)
                return jnp.sum(e * z.reshape(e.shape), axis=0)

            den = _per_head(dot_z(e_pos, pair(0)) * s_neg + dot_z(e_neg, pair(1)) * s_pos, jnp.add)
            inv = 1.0 / (den + DEN_EPS * (s_pos * s_neg))
            phi.append(_features(e_pos, e_neg, s_neg * inv, s_pos * inv))
        return phi

    def attend(phi):
        ot = jnp.concatenate([_dot(kv_acc[p], phi[p]) for p in range(NP)], axis=0)
        return ot.astype(BF16).T

    def q_step(t, carry):
        subs = [t * Q_UNROLL + s for s in range(Q_UNROLL)]
        rows = [pl.ds(pl.multiple_of(i * Q_SUB, Q_SUB), Q_SUB) for i in subs]
        feats = [query_features(_dot(wt_v[0], xn_v[r, :], _NT)) for r in rows]
        attn = [attend(f) for f in feats]
        hs = [x_v[r, :].astype(F32) + _dot(o, wo_v[...]) for r, o in zip(rows, attn)]
        for i, r, h in zip(subs, rows, hs):
            hn = _layernorm(h).astype(BF16)
            acc = h
            for c in range(F // FFN_CHUNK):
                cols = slice(c * FFN_CHUNK, (c + 1) * FFN_CHUNK)
                act = _gelu(_dot(hn, wg_v[:, cols])) * _dot(hn, wu_v[:, cols])
                acc = acc + _dot(act.astype(BF16), wd_v[cols, :])
            out_v[r, :] = acc.astype(out_v.dtype)
            out_copy(i).start()
        return carry

    lax.fori_loop(0, n2, q_step, 0)
    for i in range(n2 * Q_UNROLL):
        out_copy(i).wait()


@jax.jit
def pallas_sequential_preLN__linear_kernel_hedgehog__geglu_ffn__prompt_kernel(
    A_x: jax.Array,
    A_wqkv: jax.Array,
    A_w_phi: jax.Array,
    A_wo: jax.Array,
    B_x: jax.Array,
    B_w_gate: jax.Array,
    B_w_up: jax.Array,
    B_w_down: jax.Array,
):
    del B_x
    B, S, D = A_x.shape
    F = B_w_gate.shape[1]
    Dh = D // NUM_HEADS
    NP = NUM_HEADS // 2
    assert B == 1 and Dh == 20 and KV_SUB == LANES
    assert S % KV_SUB == 0 and (S // KV_SUB - KV_HEAD) % KV_UNROLL == 0
    assert (S // KV_SUB - KV_HEAD) // KV_UNROLL >= 2
    assert S % (Q_SUB * Q_UNROLL) == 0 and F % FFN_CHUNK == 0
    hbm = pl.BlockSpec(memory_space=pl.ANY)
    out = pl.pallas_call(
        _kernel,
        out_shape=jax.ShapeDtypeStruct((S, D), A_x.dtype),
        in_specs=[hbm] * 7,
        out_specs=hbm,
        scratch_shapes=[
            pltpu.VMEM((S, D), A_x.dtype),
            pltpu.VMEM((S, D), BF16),
            pltpu.VMEM((3, D, D), A_wqkv.dtype),
            pltpu.VMEM((3, D, D), BF16),
            pltpu.VMEM((D, D), A_wo.dtype),
            pltpu.VMEM((D, F), B_w_gate.dtype),
            pltpu.VMEM((D, F), B_w_up.dtype),
            pltpu.VMEM((F, D), B_w_down.dtype),
            pltpu.VMEM((S, D), A_x.dtype),
            pltpu.VMEM((Dh, Dh, NUM_HEADS), A_w_phi.dtype),
            pltpu.VMEM((D + NUM_HEADS, LANES), F32),
            pltpu.VMEM((NP, 2 * Dh, 4 * Dh), F32),
            pltpu.VMEM((NP, 4 * Dh, LANES), F32),
            pltpu.SemaphoreType.DMA((3,)),
            pltpu.SemaphoreType.DMA((9,)),
            pltpu.SemaphoreType.DMA((S // Q_SUB,)),
        ],
        compiler_params=pltpu.CompilerParams(vmem_limit_bytes=100 * 1024 * 1024),
    )(A_x.reshape(S, D), A_wqkv, A_w_phi.transpose(1, 2, 0), A_wo, B_w_gate, B_w_up, B_w_down)
    return out.reshape(B, S, D)
```
